```python
import jax
import jax.numpy as jnp

def _softmax(x, axis=-1):
    return jax.nn.softmax(x, axis=axis)
def _gelu(x):
    return jax.nn.gelu(x, approximate=True)
def _silu(x):
    return jax.nn.silu(x)
def _sigmoid(x):
    return jax.nn.sigmoid(x)
def _layernorm(x, axis=-1, eps=1e-5):
    m = jnp.mean(x, axis=axis, keepdims=True)
    v = jnp.var(x, axis=axis, keepdims=True)
    return (x - m) / jnp.sqrt(v + eps)
def _scatter_add(tgt, idx, src, axis=0):
    return tgt.at[idx].add(src)
def _segment_sum(src, seg, n):
    return jax.ops.segment_sum(src, seg, n)
class _Rng:
    def __init__(self, key):
        self._k = key
    def _next(self):
        self._k, sub = jax.random.split(self._k)
        return sub
    def normal(self, shape):
        return jax.random.normal(self._next(), shape, dtype=jnp.bfloat16)
    def randint(self, lo, hi, shape):
        return jax.random.randint(self._next(), shape, lo, hi, dtype=jnp.int32)
    def uniform(self, shape, lo=0.0, hi=1.0):
        return jax.random.uniform(self._next(), shape, jnp.bfloat16, lo, hi)
    def permutation(self, n):
        return jax.random.permutation(self._next(), n)


kernel_name = 'concat_heads__mha_block_cached__compressed_kv_cla__decode'

def setup_inputs():
    _rng = _Rng(jax.random.key(int.from_bytes(__import__("os").urandom(4), "little")))
    _w = (lambda a: (lambda t: t.astype(jnp.bfloat16) if jnp.issubdtype(t.dtype, jnp.floating) else t)(jnp.asarray(a)))
    def _A_setup():
        B, Sq, D = 4, 1, 576
        H, Sk, Dh = 32, 4096, 128
        return {
            "x": _w((lambda *s: _rng.normal(s) * 0.05)(B, Sq, D)),
            "k_cache": _w((lambda *s: _rng.normal(s) * 0.05)(B, H, Sk, Dh)),
            "v_cache": _w((lambda *s: _rng.normal(s) * 0.05)(B, H, Sk, Dh)),
            "wq": _w((lambda *s: _rng.normal(s) * 0.05)(D, H * Dh) * (D ** -0.5)),
            "wo": _w((lambda *s: _rng.normal(s) * 0.05)(H * Dh, D) * ((H * Dh) ** -0.5)),
        }
    _A_in = _A_setup()

    def _B_setup():
        B, H, Sq, Sk, D, M = 4, 32, 1, 4096, 128, 576
        Dc = 4 * D
        return {
            "x": _w((lambda *s: _rng.normal(s) * 0.05)(B, Sq, M)),
            "c_kv": _w((lambda *s: _rng.normal(s) * 0.05)(B, Sk, Dc)),
            "w_q": _w((lambda *s: _rng.normal(s) * 0.05)(M, H, D) * (M ** -0.5)),
            "w_uk": _w((lambda *s: _rng.normal(s) * 0.05)(Dc, H, D) * (Dc ** -0.5)),
            "w_uv": _w((lambda *s: _rng.normal(s) * 0.05)(Dc, H, D) * (Dc ** -0.5)),
            "w_o": _w((lambda *s: _rng.normal(s) * 0.05)(H, D, M) * ((H * D) ** -0.5)),
        }
    _B_in = _B_setup()

    return {
        "A_x": _A_in["x"],
        "A_k_cache": _A_in["k_cache"],
        "A_v_cache": _A_in["v_cache"],
        "A_wq": _A_in["wq"],
        "A_wo": _A_in["wo"],
        "B_x": _B_in["x"],
        "B_c_kv": _B_in["c_kv"],
        "B_w_q": _B_in["w_q"],
        "B_w_uk": _B_in["w_uk"],
        "B_w_uv": _B_in["w_uv"],
        "B_w_o": _B_in["w_o"],
    }

def reference(A_x, A_k_cache, A_v_cache, A_wq, A_wo, B_x, B_c_kv, B_w_q, B_w_uk, B_w_uv, B_w_o):
    def _A_ref(x, k_cache, v_cache, wq, wo):
        B, Sq, D = x.shape
        H, Dh = 32, 128
        q = (lambda x, *d: x.transpose(*d))((x @ wq).reshape(B, Sq, H, Dh), 0, 2, 1, 3)
        scores = jnp.einsum("bhqd,bhkd->bhqk", q, k_cache) * (Dh ** -0.5)
        p = _softmax(scores, axis=-1)
        o = jnp.einsum("bhqk,bhkd->bhqd", p, v_cache)
        return (lambda x, *d: x.transpose(*d))(o, 0, 2, 1, 3).reshape(B, Sq, H * Dh) @ wo

    def _B_ref(x, c_kv, w_q, w_uk, w_uv, w_o):
        B, Sq, M = x.shape[0], x.shape[1], x.shape[2]
        Sk = c_kv.shape[1]
        H, D = w_q.shape[1], w_q.shape[2]
        q = jnp.einsum("bqm,mhd->bhqd", x, w_q)
        k = jnp.einsum("bkc,chd->bhkd", c_kv, w_uk)
        v = jnp.einsum("bkc,chd->bhkd", c_kv, w_uv)
        scores = jnp.einsum("bhqd,bhkd->bhqk", q, k) * (D ** -0.5)
        off = Sk - Sq
        qi = jnp.arange(Sq)[:, None]
        kj = jnp.arange(Sk)[None, :]
        cmask = kj <= (qi + off)
        scores = jnp.where(cmask[None, None], scores, -1e9)
        p = _softmax(scores, axis=-1)
        ctx = jnp.einsum("bhqk,bhkd->bhqd", p, v)
        return jnp.einsum("bhqd,hdm->bqm", ctx, w_o)

    a = _A_ref(A_x, A_k_cache, A_v_cache, A_wq, A_wo)
    b = _B_ref(B_x, B_c_kv, B_w_q, B_w_uk, B_w_uv, B_w_o)
    return jnp.concatenate([a, b], axis=-1)
```

```python
import jax
import jax.numpy as jnp
import jax.experimental.pallas as pl
import jax.experimental.pallas.tpu as pltpu

_NT = (((1,), (1,)), ((), ()))
_NN = (((1,), (0,)), ((), ()))
_F32 = jnp.float32
_BF16 = jnp.bfloat16

_NBUF = 4


def _dot(a, b, dims):
    return jax.lax.dot_general(a, b, dims, preferred_element_type=_F32)


def _split_heads(src_ref, dst_ref, i, heads):
    _, rows, D = src_ref.shape
    n = rows // heads
    words_ref = src_ref.bitcast(jnp.uint32)
    dst_rows = pl.ds(pl.multiple_of(i * n, n), n)
    for j in range(heads // 2):
        words = words_ref[i, pl.ds(j, n, stride=heads // 2), :]
        lo = pltpu.bitcast(words << 16, _F32)
        hi = pltpu.bitcast(words & jnp.uint32(0xFFFF0000), _F32)
        dst_ref[dst_rows, 2 * j * D:(2 * j + 1) * D] = lo.astype(_BF16)
        dst_ref[dst_rows, (2 * j + 1) * D:(2 * j + 2) * D] = hi.astype(_BF16)


def _kernel(
    ax_hbm, k_hbm, v_hbm, awq_hbm, awo_hbm,
    bx_hbm, ckv_hbm, bwq_hbm, uk_hbm, uv_hbm, bwo_hbm,
    out_ref,
    ax_v, bx_v, awq_v, awo_v, ckv_v, bwq_v, uk_v, uv_v, bwo_v,
    k_v, v_v, w2d_v, qa_v, qb_v, lat_v,
    w_sem, c_sem, kv_sem,
    *, B, H, S, D, M, C,
):
    scale = D ** -0.5

    def wcopy(i, src, dst):
        return pltpu.make_async_copy(src, dst, w_sem.at[i])

    cp_ax = wcopy(0, ax_hbm, ax_v)
    cp_bx = wcopy(1, bx_hbm, bx_v)
    cp_bwq = wcopy(2, bwq_hbm, bwq_v)
    cp_uk = wcopy(3, uk_hbm, uk_v)
    cp_uv = wcopy(4, uv_hbm, uv_v)
    cp_bwo = wcopy(5, bwo_hbm, bwo_v)
    cp_awq = wcopy(6, awq_hbm, awq_v)
    cp_awo = wcopy(7, awo_hbm, awo_v)

    def cp_ckv(b):
        return pltpu.make_async_copy(ckv_hbm.at[b], ckv_v.at[b], c_sem.at[b])

    def kv_copies(t, slot):
        return (
            pltpu.make_async_copy(k_hbm.at[t], k_v.at[slot], kv_sem.at[0, slot]),
            pltpu.make_async_copy(v_hbm.at[t], v_v.at[slot], kv_sem.at[1, slot]),
        )

    cp_bx.start()
    cp_ax.start()
    cp_bwq.start()
    cp_uk.start()
    for b in range(B):
        cp_ckv(b).start()
    cp_uv.start()
    cp_bwo.start()
    cp_awq.start()
    cp_awo.start()
    for t in range(_NBUF):
        for cp in kv_copies(t, t):
            cp.start()

    cp_bx.wait()
    cp_bwq.wait()

    @pl.loop(0, bwq_v.shape[0])
    def _(i):
        _split_heads(bwq_v, w2d_v, i, H)

    qb = _dot(bx_v[...], w2d_v[...], _NN)
    for h in range(H):
        qb_v[h] = qb[:, h * D:(h + 1) * D]

    cp_uk.wait()

    @pl.loop(0, uk_v.shape[0])
    def _(i):
        _split_heads(uk_v, w2d_v, i, H)

    @pl.loop(0, H)
    def _(h):
        w = w2d_v[:C, pl.ds(pl.multiple_of(h * D, D), D)]
        r = _dot(qb_v[h].astype(_BF16), w, _NT)
        for b in range(B):
            lat_v[pl.ds(b * H + h, 1), :] = r[b:b + 1]

    @pl.loop(0, B)
    def _(b):
        cp_ckv(b).wait()
        rows = pl.ds(pl.multiple_of(b * H, H), H)
        s = _dot(lat_v[rows, :].astype(_BF16), ckv_v[b], _NT) * scale
        p = jnp.exp(s - jnp.max(s, axis=-1, keepdims=True))
        l = jnp.sum(p, axis=-1, keepdims=True)
        lat_v[rows, :] = _dot(p.astype(_BF16), ckv_v[b], _NN) / l

    cp_uv.wait()

    @pl.loop(0, uv_v.shape[0])
    def _(i):
        _split_heads(uv_v, w2d_v, i, H)

    cp_bwo.wait()

    def b_out(h, acc):
        w = w2d_v[:C, pl.ds(pl.multiple_of(h * D, D), D)]
        cc = jnp.concatenate(
            [lat_v[pl.ds(b * H + h, 1), :] for b in range(B)], axis=0)
        ctx = _dot(cc.astype(_BF16), w, _NN)
        return acc + _dot(ctx.astype(_BF16), bwo_v[h], _NT)

    out_b = jax.lax.fori_loop(0, H, b_out, jnp.zeros((B, M), _F32))

    cp_ax.wait()
    cp_awq.wait()
    qa = _dot(ax_v[...], awq_v[...], _NN)
    for h in range(H):
        qa_v[h] = qa[:, h * D:(h + 1) * D]
    cp_awo.wait()

    def a_step(t, acc):
        b = t // H
        h = t % H
        slot = t % _NBUF
        cp_k, cp_v = kv_copies(t, slot)
        nxt_k, nxt_v = kv_copies(jnp.minimum(t + _NBUF, B * H - 1), slot)
        cp_k.wait()
        s = _dot(qa_v[h].astype(_BF16), k_v[slot], _NT) * scale
        pl.when(t + _NBUF < B * H)(nxt_k.start)
        p = jnp.exp(s - jnp.max(s, axis=-1, keepdims=True))
        l = jnp.sum(p, axis=-1, keepdims=True)
        cp_v.wait()
        o = _dot(p.astype(_BF16), v_v[slot], _NN) / l
        pl.when(t + _NBUF < B * H)(nxt_v.start)
        row = jax.lax.broadcasted_iota(jnp.int32, o.shape, 0)
        o = jnp.where(row == b, o, 0.0)
        wo = awo_v[:, pl.ds(pl.multiple_of(h * D, D), D)]
        return acc + _dot(o.astype(_BF16), wo, _NT)

    out_a = jax.lax.fori_loop(0, B * H, a_step, jnp.zeros((B, M), _F32))
    out_ref[...] = jnp.concatenate([out_a, out_b], axis=-1).astype(out_ref.dtype)


@jax.jit
def pallas_concat_heads__mha_block_cached__compressed_kv_cla__decode_kernel(
    A_x: jax.Array,
    A_k_cache: jax.Array,
    A_v_cache: jax.Array,
    A_wq: jax.Array,
    A_wo: jax.Array,
    B_x: jax.Array,
    B_c_kv: jax.Array,
    B_w_q: jax.Array,
    B_w_uk: jax.Array,
    B_w_uv: jax.Array,
    B_w_o: jax.Array,
):
    B, H, S, D = A_k_cache.shape
    M = A_x.shape[-1]
    C = B_c_kv.shape[-1]
    R = 64

    def kernel(*refs):
        _kernel(*refs, B=B, H=H, S=S, D=D, M=M, C=C)

    vmem = pltpu.VMEM
    out = pl.pallas_call(
        kernel,
        out_shape=jax.ShapeDtypeStruct((B, 2 * M), A_x.dtype),
        in_specs=[pl.BlockSpec(memory_space=pltpu.HBM)] * 11,
        out_specs=pl.BlockSpec(memory_space=vmem),
        scratch_shapes=[
            vmem((B, M), _BF16),
            vmem((B, M), _BF16),
            vmem((M, H * D), _BF16),
            vmem((M, H * D), _BF16),
            vmem((B, S, C), _BF16),
            vmem((M // R, R * H, D), _BF16),
            vmem((C // R, R * H, D), _BF16),
            vmem((C // R, R * H, D), _BF16),
            vmem((H, M, D), _BF16),
            vmem((_NBUF, S, D), _BF16),
            vmem((_NBUF, S, D), _BF16),
            vmem((M, H * D), _BF16),
            vmem((H, B, D), _F32),
            vmem((H, B, D), _F32),
            vmem((B * H, C), _F32),
            pltpu.SemaphoreType.DMA((8,)),
            pltpu.SemaphoreType.DMA((B,)),
            pltpu.SemaphoreType.DMA((2, _NBUF)),
        ],
        compiler_params=pltpu.CompilerParams(vmem_limit_bytes=100 * 1024 * 1024),
    )(
        A_x.reshape(B, M),
        A_k_cache.reshape(B * H, S, D),
        A_v_cache.reshape(B * H, S, D),
        A_wq,
        A_wo.T,
        B_x.reshape(B, M),
        B_c_kv,
        B_w_q.reshape(M // R, R * H, D),
        B_w_uk.reshape(C // R, R * H, D),
        B_w_uv.reshape(C // R, R * H, D),
        B_w_o.transpose(0, 2, 1),
    )
    return out.reshape(B, 1, 2 * M)
```

```python
import jax
import jax.numpy as jnp
import jax.experimental.pallas as pl
import jax.experimental.pallas.tpu as pltpu

_NT = (((1,), (1,)), ((), ()))
_NN = (((1,), (0,)), ((), ()))
_F32 = jnp.float32
_BF16 = jnp.bfloat16

_G = 16
_T = 512
_PR = 64
_PN = 2
_AHEAD = 2
_R = 64
_FRONT = 0
_SEMCHK = True


def _dot(a, b, dims):
    return jax.lax.dot_general(a, b, dims, preferred_element_type=_F32)


def _ds(i, n):
    return pl.ds(pl.multiple_of(i * n, n), n)


def _split_heads(src_ref, dst_ref, i, heads):
    _, rows, D = src_ref.shape
    n = rows // heads
    words_ref = src_ref.bitcast(jnp.uint32)
    for j in range(heads // 2):
        words = words_ref[i, pl.ds(j, n, stride=heads // 2), :]
        lo = pltpu.bitcast(words << 16, _F32)
        hi = pltpu.bitcast(words & jnp.uint32(0xFFFF0000), _F32)
        dst_ref[_ds(i, n), 2 * j * D:(2 * j + 1) * D] = lo.astype(_BF16)
        dst_ref[_ds(i, n), (2 * j + 1) * D:(2 * j + 2) * D] = hi.astype(_BF16)


def _kernel(
    ax_hbm, k_hbm, v_hbm, awq_hbm, awo_hbm,
    bx_hbm, ckv_hbm, bwq_hbm, uk_hbm, uv_hbm, bwo_hbm,
    out_ref,
    ax_v, bx_v, awq_v, awo_v, ckv_v, bwq_v, uk_v, uv_v, bwo_v,
    ring_v, w2d_v, qa_v, sa_v, oa_v, qb_v, lat_v, pb_v, ob_v,
    sems,
    *, B, H, S, D, M, C,
):
    scale = D ** -0.5
    nslot = _AHEAD + 1
    nchunk = S // _T
    nstep = B * H // _G * nchunk

    (SEM_AX, SEM_BX, SEM_AWQ, SEM_CKV, SEM_BWQ, SEM_UK, SEM_UV, SEM_BWO,
     SEM_RING) = range(9)
    SEM_AWO = SEM_RING + nslot

    def start(src, dst, idx, sem, prio):
        pltpu.make_async_copy(src.at[idx], dst.at[idx], sems.at[sem]).start(
            priority=prio)

    def wait(dst, sem):
        pltpu.make_async_copy(dst, dst, sems.at[sem]).wait()

    def start_kv(src, t, slot):
        g = t // nchunk
        c = t % nchunk

        @pl.loop(0, _T // _PR)
        def _(r):
            for j in range(_G // _PN):
                pltpu.make_async_copy(
                    src.at[pl.ds(g * _G + j * _PN, _PN),
                           _ds(c * (_T // _PR) + r, _PR)],
                    ring_v.at[slot, pl.ds(j * _PN, _PN), _ds(r, _PR)],
                    sems.at[SEM_RING + slot],
                ).start(priority=j % 2)

    def start_awo(i, n):
        @pl.loop(0, _R // 8)
        def _(r):
            w = 2048 // n
            for j in range(H * D // w):
                start(awo_hbm, awo_v,
                      (pl.ds(i, n), _ds(r, 8), pl.ds(j * w, w)),
                      SEM_AWO + i // 2, j % 2)

    pltpu.make_async_copy(ax_hbm, ax_v, sems.at[SEM_AX]).start()
    pltpu.make_async_copy(bx_hbm, bx_v, sems.at[SEM_BX]).start()

    if _FRONT == 0:
        @pl.loop(0, _R // 8)
        def _(r):
            for q in range(4):
                for j in range(3):
                    start(awq_hbm, awq_v,
                          (pl.ds(3 * j, 3), _ds(r, 8), pl.ds(q * 1024, 1024)),
                          SEM_AWQ, 0)
                    start(bwq_hbm, bwq_v, (pl.ds(3 * j, 3), _ds(4 * r + q, 64)),
                          SEM_BWQ, 1)

        @pl.loop(0, _R * H // 64)
        def _(r):
            for j in range(4):
                start(uk_hbm, uk_v, (pl.ds(2 * j, 2), _ds(r, 64)), SEM_UK, 0)
                start(uv_hbm, uv_v, (pl.ds(2 * j, 2), _ds(r, 64)), SEM_UV, 1)

        @pl.loop(0, ckv_v.shape[1] // 16)
        def _(r):
            for j in range(8):
                start(ckv_hbm, ckv_v, (pl.ds(2 * j, 2), _ds(r, 16)), SEM_CKV, j % 2)

        @pl.loop(0, bwo_v.shape[1] // 64)
        def _(r):
            for j in range(4):
                start(bwo_hbm, bwo_v, (pl.ds(2 * j, 2), _ds(r, 64)), SEM_BWO, j % 2)
    else:
        for src, dst, sem in ((awq_hbm, awq_v, SEM_AWQ), (bwq_hbm, bwq_v, SEM_BWQ),
                              (uk_hbm, uk_v, SEM_UK), (uv_hbm, uv_v, SEM_UV),
                              (ckv_hbm, ckv_v, SEM_CKV), (bwo_hbm, bwo_v, SEM_BWO)):
            pltpu.make_async_copy(src, dst, sems.at[sem]).start()

    wait(ax_v, SEM_AX)
    wait(awq_v, SEM_AWQ)
    qa = _dot(ax_v[...], awq_v[...].reshape(M, H * D), _NN)
    for h in range(H):
        qa_v[pl.ds(h, B, stride=H), :] = qa[:, h * D:(h + 1) * D]

    @pl.loop(0, _AHEAD)
    def _(t):
        start_kv(k_hbm, t, t)

    wait(bx_v, SEM_BX)
    wait(bwq_v, SEM_BWQ)
    wait(uk_v, SEM_UK)
    wait(uv_v, SEM_UV)
    wait(ckv_v, SEM_CKV)
    wait(bwo_v, SEM_BWO)
    ob_v[...] = jnp.zeros_like(ob_v)

    def b_query(_):
        qb = _dot(bx_v[...], w2d_v[...], _NN)
        for h in range(H):
            qb_v[h] = qb[:, h * D:(h + 1) * D]

    def b_absorb(h):
        r = _dot(qb_v[h].astype(_BF16), w2d_v[:C, _ds(h, D)], _NT)
        for b in range(B):
            lat_v[pl.ds(b * H + h, 1), :] = r[b:b + 1]

    def ckv(b):
        n = ckv_v.shape[0] // B
        return ckv_v[pl.ds(b * n, n)].reshape(S, C)

    def b_probs(b):
        s = _dot(lat_v[_ds(b, H), :].astype(_BF16), ckv(b), _NT) * scale
        p = jnp.exp(s - jnp.max(s, axis=-1, keepdims=True))
        pb_v[b] = (p / jnp.sum(p, axis=-1, keepdims=True)).astype(_BF16)

    def b_context(b):
        lat_v[_ds(b, H), :] = _dot(pb_v[b], ckv(b), _NN)

    def b_output(h):
        cc = jnp.concatenate(
            [lat_v[pl.ds(b * H + h, 1), :] for b in range(B)], axis=0)
        ctx = _dot(cc.astype(_BF16), w2d_v[:C, _ds(h, D)], _NN)
        n = H // bwo_v.shape[0]
        wo = bwo_v[h // n, pl.ds(pl.multiple_of(h % n * M, 64), M), :]
        ob_v[...] += _dot(ctx.astype(_BF16), wo, _NT)

    def run_pieces(t, pieces):
        lo = 0
        for n, fn in pieces:
            pl.when(jnp.logical_and(t >= lo, t < lo + n))(
                lambda fn=fn, lo=lo: fn(t - lo))
            lo += n
        assert lo <= nstep

    @pl.loop(0, nstep)
    def _(t):
        nxt = t + _AHEAD
        pl.when(nxt < nstep)(lambda: start_kv(k_hbm, nxt, nxt % nslot))
        pl.when(nxt >= nstep)(lambda: start_kv(v_hbm, nxt - nstep, nxt % nslot))
        slot = t % nslot
        wait(ring_v.at[slot], SEM_RING + slot)
        q = qa_v[_ds(t // nchunk, _G), :].astype(_BF16)
        row = jax.lax.broadcasted_iota(jnp.int32, (_G, _T), 0)
        s = _dot(q, ring_v[slot, 0], _NT)
        for i in range(1, _G):
            s = jnp.where(row == i, _dot(q, ring_v[slot, i], _NT), s)
        sa_v[t] = s * scale
        run_pieces(t, [
            (M // _R, lambda i: _split_heads(bwq_v, w2d_v, i, H)),
            (1, b_query),
            (C // _R, lambda i: _split_heads(uk_v, w2d_v, i, H)),
            (H, b_absorb),
        ])

    def v_step(t, carry):
        acc, l = carry
        nxt = t + _AHEAD
        pl.when(nxt < nstep)(lambda: start_kv(v_hbm, nxt, (nxt + nstep) % nslot))
        pl.when(nxt >= nstep)(lambda: start_awo(2 * (nxt - nstep), 2))
        g = t // nchunk
        first = t % nchunk == 0
        m = jnp.max(jnp.max(sa_v[pl.ds(g * nchunk, nchunk)], axis=0),
                    axis=-1, keepdims=True)
        p = jnp.exp(sa_v[t] - m)
        l = jnp.where(first, 0.0, l) + jnp.sum(p, axis=-1, keepdims=True)
        p = p.astype(_BF16)
        slot = (t + nstep) % nslot
        wait(ring_v.at[slot], SEM_RING + slot)
        row = jax.lax.broadcasted_iota(jnp.int32, (_G, D), 0)
        o = _dot(p, ring_v[slot, 0], _NN)
        for i in range(1, _G):
            o = jnp.where(row == i, _dot(p, ring_v[slot, i], _NN), o)
        acc = jnp.where(first, 0.0, acc) + o

        @pl.when(t % nchunk == nchunk - 1)
        def _():
            oa_v[_ds(g, _G), :] = acc / l

        run_pieces(t, [
            (B, b_probs),
            (B, b_context),
            (C // _R, lambda i: _split_heads(uv_v, w2d_v, i, H)),
            (H, b_output),
        ])
        return acc, l

    jax.lax.fori_loop(0, nstep, v_step,
                      (jnp.zeros((_G, D), _F32), jnp.zeros((_G, 1), _F32)))

    nwo = M // _R
    for i in range(2 * _AHEAD, nwo, 2):
        start_awo(i, min(2, nwo - i))
    oa = jnp.concatenate(
        [oa_v[pl.ds(h, B, stride=H), :] for h in range(H)], axis=-1).astype(_BF16)
    outs = []
    for i in range(0, nwo, 2):
        n = min(2, nwo - i)
        wait(awo_v.at[pl.ds(i, n)], SEM_AWO + i // 2)
        outs.append(_dot(oa, awo_v[pl.ds(i, n)].reshape(n * _R, H * D), _NT))
    out_ref[...] = jnp.concatenate(outs + [ob_v[...]], axis=-1).astype(out_ref.dtype)


@jax.jit
def pallas_concat_heads__mha_block_cached__compressed_kv_cla__decode_kernel(
    A_x: jax.Array,
    A_k_cache: jax.Array,
    A_v_cache: jax.Array,
    A_wq: jax.Array,
    A_wo: jax.Array,
    B_x: jax.Array,
    B_c_kv: jax.Array,
    B_w_q: jax.Array,
    B_w_uk: jax.Array,
    B_w_uv: jax.Array,
    B_w_o: jax.Array,
):
    B, H, S, D = A_k_cache.shape
    M = A_x.shape[-1]
    C = B_c_kv.shape[-1]

    def kernel(*refs):
        _kernel(*refs, B=B, H=H, S=S, D=D, M=M, C=C)

    ax = A_x.reshape(B, M)
    k = A_k_cache.reshape(B * H, S, D)
    v = A_v_cache.reshape(B * H, S, D)
    awq = A_wq.reshape(M // _R, _R, H * D)
    awo = A_wo.T.reshape(M // _R, _R, H * D)
    bx = B_x.reshape(B, M)
    ckv = B_c_kv.reshape(4 * B, S // 4, C)
    bwq = B_w_q.reshape(M // _R, _R * H, D)
    uk = B_w_uk.reshape(C // _R, _R * H, D)
    uv = B_w_uv.reshape(C // _R, _R * H, D)
    bwo = B_w_o.transpose(0, 2, 1).reshape(8, H // 8 * M, D)

    vmem = pltpu.VMEM
    nstep = B * H // _G * (S // _T)
    out = pl.pallas_call(
        kernel,
        out_shape=jax.ShapeDtypeStruct((B, 2 * M), A_x.dtype),
        in_specs=[pl.BlockSpec(memory_space=pltpu.HBM)] * 11,
        out_specs=pl.BlockSpec(memory_space=vmem),
        scratch_shapes=[
            *[vmem(a.shape, a.dtype)
              for a in (ax, bx, awq, awo, ckv, bwq, uk, uv, bwo)],
            vmem((_AHEAD + 1, _G, _T, D), _BF16),
            vmem((M, H * D), _BF16),
            vmem((B * H, D), _F32),
            vmem((nstep, _G, _T), _F32),
            vmem((B * H, D), _F32),
            vmem((H, B, D), _F32),
            vmem((B * H, C), _F32),
            vmem((B, H, S), _BF16),
            vmem((B, M), _F32),
            pltpu.SemaphoreType.DMA((8 + _AHEAD + 1 + (M // _R + 1) // 2,)),
        ],
        compiler_params=pltpu.CompilerParams(
            vmem_limit_bytes=100 * 1024 * 1024,
            disable_semaphore_checks=not _SEMCHK),
    )(ax, k, v, awq, awo, bx, ckv, bwq, uk, uv, bwo)
    return out.reshape(B, 1, 2 * M)
```

```python
import jax
import jax.numpy as jnp
import jax.experimental.pallas as pl
import jax.experimental.pallas.tpu as pltpu
import numpy as np

_NT = (((1,), (1,)), ((), ()))
_NN = (((1,), (0,)), ((), ()))
_F32 = jnp.float32
_BF16 = jnp.bfloat16
_ALL = slice(None)

B, H, S, D, M, C = 4, 32, 4096, 128, 576, 512

_G = 16
_T = 512
_AHEAD = 3
_R = 64
_NSLOT = _AHEAD + 1
_NCHUNK = S // _T
_NSTEP = B * H // _G * _NCHUNK
_FAN = ((0, 6, 1), (12, 2, 0), (6, 6, 1), (14, 2, 0))
_WO_PARTS = ((0, 6), (6, 2), (8, 1))


def _dot(a, b, dims):
    return jax.lax.dot_general(a, b, dims, preferred_element_type=_F32)


def _ds(i, n):
    return pl.ds(pl.multiple_of(i * n, n), n)


def _start(src, dst, idx, sem, priority):
    pltpu.make_async_copy(src.at[idx], dst.at[idx], sem).start(priority=priority)


def _wait(dst, sem):
    pltpu.make_async_copy(dst, dst, sem).wait()


def _split_heads(src_ref, dst_ref, i):
    inner = src_ref.shape[1]
    words_ref = src_ref.bitcast(jnp.uint32)
    for j in range(H // 2):
        words = words_ref[i // inner, i % inner, pl.ds(j, _R, stride=H // 2), :]
        lo = pltpu.bitcast(words << 16, _F32)
        hi = pltpu.bitcast(words & np.uint32(0xFFFF0000), _F32)
        dst_ref[_ds(i, _R), 2 * j * D:(2 * j + 1) * D] = lo.astype(_BF16)
        dst_ref[_ds(i, _R), (2 * j + 1) * D:(2 * j + 2) * D] = hi.astype(_BF16)


def _run_pieces(t, pieces):
    first = 0
    for n, every, fn in pieces:
        i = t - first
        pl.when((i >= 0) & (i < n * every) & (i % every == 0))(
            lambda fn=fn, i=i, every=every: fn(i // every))
        first += n * every
    assert first <= _NSTEP


def _kernel(
    ax_hbm, k_hbm, v_hbm, awq_hbm, awo_hbm,
    bx_hbm, ckv_hbm, bwq_hbm, uk_hbm, uv_hbm, bwo_hbm,
    out_ref,
    awq_v, awo_v, ckv_v, bwq_v, uk_v, uv_v, bwo_v,
    ring_v, w2d_v, qa_v, sa_v, oa_v, qb_v, lat_v, pb_v, ob_v, ax_v, bx_v,
    wo_sems,
):
    scale = D ** -0.5

    def b_query(_):
        q = _dot(bx_v[...], w2d_v[...], _NN)
        for h in range(H):
            qb_v[h] = q[:, h * D:(h + 1) * D]

    def b_absorb(h):
        r = _dot(qb_v[h].astype(_BF16), w2d_v[:C, _ds(h, D)], _NT)
        for b in range(B):
            lat_v[pl.ds(b * H + h, 1), :] = r[b:b + 1]

    def ckv(b):
        n = ckv_v.shape[0] // B
        return ckv_v[pl.ds(b * n, n)].reshape(S, C)

    def b_probs(b):
        s = _dot(lat_v[_ds(b, H), :].astype(_BF16), ckv(b), _NT) * scale
        p = jnp.exp(s - jnp.max(s, axis=-1, keepdims=True))
        pb_v[b] = (p / jnp.sum(p, axis=-1, keepdims=True)).astype(_BF16)

    def b_context(b):
        lat_v[_ds(b, H), :] = _dot(pb_v[b], ckv(b), _NN)

    def b_output(h):
        lat = jnp.concatenate(
            [lat_v[pl.ds(b * H + h, 1), :] for b in range(B)], axis=0)
        ctx = _dot(lat.astype(_BF16), w2d_v[:C, _ds(h, D)], _NN)
        n = H // bwo_v.shape[0]
        wo = bwo_v[h // n, pl.ds(pl.multiple_of(h % n * M, 64), M), :]
        ob_v[...] += _dot(ctx.astype(_BF16), wo, _NT)

    def start_wo():
        @pl.loop(0, _R // 8)
        def _(r):
            for q in range(4):
                piece = (_ds(r, 8), pl.ds(q * 1024, 1024))
                _start(awo_hbm, awo_v, (pl.ds(0, 4), *piece), wo_sems.at[0], 1)
                _start(awo_hbm, awo_v, (pl.ds(4, 2), *piece), wo_sems.at[0], 0)

        for j in (1, 2):
            _start(awo_hbm, awo_v, pl.ds(*_WO_PARTS[j]), wo_sems.at[j], 1)

    def stream(sems):
        s_ax, s_bx, s_awq, s_ckv, s_bwq, s_uk, s_uv, s_bwo = (
            sems.at[_NSLOT + i] for i in range(8))

        def start_kv(src, t, slot):
            g, c = t // _NCHUNK, t % _NCHUNK

            @pl.loop(0, _T // 64)
            def _(r):
                for i, n, priority in _FAN:
                    pltpu.make_async_copy(
                        src.at[pl.ds(g * _G + i, n), _ds(c * (_T // 64) + r, 64)],
                        ring_v.at[slot, pl.ds(i, n), _ds(r, 64)],
                        sems.at[slot],
                    ).start(priority=priority)

        pltpu.make_async_copy(ax_hbm, ax_v, s_ax).start()
        pltpu.make_async_copy(bx_hbm, bx_v, s_bx).start()

        @pl.loop(0, 24)
        def _(r):
            for q in range(4):
                p = 4 * r + q
                _start(awq_hbm, awq_v,
                       (_ALL, _ds(r, 8), pl.ds(q * 1024, 1024)), s_awq, 1)
                _start(bwo_hbm, bwo_v, (0, _ds(p, 64)), s_bwo, 0)
                _start(bwq_hbm, bwq_v, (_ALL, p // 32, _ds(p % 32, 64)), s_bwq, 1)
                _start(bwo_hbm, bwo_v, (1, _ds(p, 64)), s_bwo, 0)

        @pl.loop(0, 48)
        def _(p):
            _start(uk_hbm, uk_v, (_ALL, p // 32, _ds(p % 32, 64)), s_uk, 1)
            _start(bwo_hbm, bwo_v, (0, _ds(96 + p, 64)), s_bwo, 0)
            _start(uv_hbm, uv_v, (_ALL, p // 32, _ds(p % 32, 64)), s_uv, 1)
            _start(bwo_hbm, bwo_v, (1, _ds(96 + p, 64)), s_bwo, 0)

        @pl.loop(48, 64)
        def _(p):
            for src, dst, sem in ((uk_hbm, uk_v, s_uk), (uv_hbm, uv_v, s_uv)):
                _start(src, dst, (pl.ds(0, 3), p // 32, _ds(p % 32, 64)), sem, 1)
                _start(src, dst, (3, p // 32, _ds(p % 32, 64)), sem, 0)

        @pl.loop(0, 64)
        def _(p):
            for i, n, priority in _FAN:
                _start(ckv_hbm, ckv_v, (pl.ds(i, n), _ds(p, 16)), s_ckv, priority)

        _wait(ax_v, s_ax)
        _wait(awq_v, s_awq)
        q = _dot(ax_v[...], awq_v[...].reshape(M, H * D), _NN)
        for h in range(H):
            qa_v[pl.ds(h, B, stride=H), :] = q[:, h * D:(h + 1) * D]

        @pl.loop(0, _AHEAD)
        def _(t):
            start_kv(k_hbm, t, t)

        _wait(bx_v, s_bx)
        _wait(bwq_v, s_bwq)
        _wait(uk_v, s_uk)
        _wait(uv_v, s_uv)
        _wait(bwo_v, s_bwo)
        _wait(ckv_v, s_ckv)
        ob_v[...] = jnp.zeros(ob_v.shape, ob_v.dtype)

        def each_own_head(lhs, slot, dims):
            out = _dot(lhs, ring_v[slot, 0], dims)
            row = jax.lax.broadcasted_iota(jnp.int32, out.shape, 0)
            for i in range(1, _G):
                out = jnp.where(row == i, _dot(lhs, ring_v[slot, i], dims), out)
            return out

        @pl.loop(0, _NSTEP)
        def _(t):
            nxt = t + _AHEAD
            pl.when(nxt < _NSTEP)(lambda: start_kv(k_hbm, nxt, nxt % _NSLOT))
            pl.when(nxt >= _NSTEP)(
                lambda: start_kv(v_hbm, nxt - _NSTEP, nxt % _NSLOT))
            slot = t % _NSLOT
            _wait(ring_v.at[slot], sems.at[slot])
            q = qa_v[_ds(t // _NCHUNK, _G), :].astype(_BF16)
            sa_v[t] = each_own_head(q, slot, _NT) * scale
            _run_pieces(t, [
                (M // _R, 1, lambda i: _split_heads(bwq_v, w2d_v, i)),
                (1, 1, b_query),
                (C // _R, 1, lambda i: _split_heads(uk_v, w2d_v, i)),
                (H, 1, b_absorb),
            ])

        def v_step(t, carry):
            acc, l = carry
            nxt = t + _AHEAD
            pl.when(nxt < _NSTEP)(
                lambda: start_kv(v_hbm, nxt, (_NSTEP + nxt) % _NSLOT))
            pl.when(nxt == _NSTEP)(start_wo)
            g, c = t // _NCHUNK, t % _NCHUNK
            m = jnp.max(jnp.max(sa_v[pl.ds(g * _NCHUNK, _NCHUNK)], axis=0),
                        axis=-1, keepdims=True)
            p = jnp.exp(sa_v[t] - m)
            l = jnp.where(c == 0, 0.0, l) + jnp.sum(p, axis=-1, keepdims=True)
            slot = (_NSTEP + t) % _NSLOT
            _wait(ring_v.at[slot], sems.at[slot])
            acc = (jnp.where(c == 0, 0.0, acc)
                   + each_own_head(p.astype(_BF16), slot, _NN))

            @pl.when(c == _NCHUNK - 1)
            def _():
                oa_v[_ds(g, _G), :] = acc / l

            _run_pieces(t, [
                (B, 2, b_probs),
                (B, 1, b_context),
                (C // _R, 1, lambda i: _split_heads(uv_v, w2d_v, i)),
                (H, 1, b_output),
            ])
            return acc, l

        jax.lax.fori_loop(0, _NSTEP, v_step,
                          (jnp.zeros((_G, D), _F32), jnp.zeros((_G, 1), _F32)))

    pl.run_scoped(stream, pltpu.SemaphoreType.DMA((_NSLOT + 8,)))

    o = jnp.concatenate(
        [oa_v[pl.ds(h, B, stride=H), :] for h in range(H)], axis=-1).astype(_BF16)
    outs = []
    for j, (i, n) in enumerate(_WO_PARTS):
        _wait(awo_v.at[pl.ds(i, n)], wo_sems.at[j])
        outs.append(_dot(o, awo_v[pl.ds(i, n)].reshape(n * _R, H * D), _NT))
    out_ref[...] = jnp.concatenate(outs + [ob_v[...]], axis=-1).astype(out_ref.dtype)


@jax.jit
def pallas_concat_heads__mha_block_cached__compressed_kv_cla__decode_kernel(
    A_x: jax.Array,
    A_k_cache: jax.Array,
    A_v_cache: jax.Array,
    A_wq: jax.Array,
    A_wo: jax.Array,
    B_x: jax.Array,
    B_c_kv: jax.Array,
    B_w_q: jax.Array,
    B_w_uk: jax.Array,
    B_w_uv: jax.Array,
    B_w_o: jax.Array,
):
    assert A_x.shape == B_x.shape == (B, 1, M)
    assert A_k_cache.shape == A_v_cache.shape == (B, H, S, D)
    assert B_c_kv.shape == (B, S, C)

    ax = A_x.reshape(B, M)
    k = A_k_cache.reshape(B * H, S, D)
    v = A_v_cache.reshape(B * H, S, D)
    awq = A_wq.reshape(3, M // 3, H * D)
    awo = A_wo.T.reshape(M // _R, _R, H * D)
    bx = B_x.reshape(B, M)
    ckv = B_c_kv.reshape(4 * B, S // 4, C)
    bwq = B_w_q.reshape(3, M // _R // 3, _R * H, D)
    uk = B_w_uk.reshape(4, C // _R // 4, _R * H, D)
    uv = B_w_uv.reshape(4, C // _R // 4, _R * H, D)
    bwo = B_w_o.transpose(0, 2, 1).reshape(2, H // 2 * M, D)

    vmem = pltpu.VMEM
    out = pl.pallas_call(
        _kernel,
        out_shape=jax.ShapeDtypeStruct((B, 2 * M), A_x.dtype),
        in_specs=[pl.BlockSpec(memory_space=pltpu.HBM)] * 11,
        out_specs=pl.BlockSpec(memory_space=vmem),
        scratch_shapes=[
            *[vmem(a.shape, _BF16) for a in (awq, awo, ckv, bwq, uk, uv, bwo)],
            vmem((_NSLOT, _G, _T, D), _BF16),
            vmem((M, H * D), _BF16),
            vmem((B * H, D), _F32),
            vmem((_NSTEP, _G, _T), _F32),
            vmem((B * H, D), _F32),
            vmem((H, B, D), _F32),
            vmem((B * H, C), _F32),
            vmem((B, H, S), _BF16),
            vmem((B, M), _F32),
            vmem((B, M), _BF16),
            vmem((B, M), _BF16),
            pltpu.SemaphoreType.DMA((len(_WO_PARTS),)),
        ],
        compiler_params=pltpu.CompilerParams(vmem_limit_bytes=100 * 1024 * 1024),
    )(ax, k, v, awq, awo, bx, ckv, bwq, uk, uv, bwo)
    return out.reshape(B, 1, 2 * M)
```

```python
import jax
import jax.numpy as jnp
import jax.experimental.pallas as pl
import jax.experimental.pallas.tpu as pltpu

_NT = (((1,), (1,)), ((), ()))
_NN = (((1,), (0,)), ((), ()))
_F32 = jnp.float32
_BF16 = jnp.bfloat16
_ALL = slice(None)

B, H, S, D, M, C = 4, 32, 4096, 128, 576, 512

_G = 16
_T = 512
_AHEAD = 3
_R = 64
_NSLOT = _AHEAD + 1
_NCHUNK = S // _T
_NSTEP = B * H // _G * _NCHUNK
_FAN = ((0, 4, 1), (11, 2, 0), (4, 4, 1), (13, 2, 0), (8, 3, 1), (15, 1, 0))
_WO_PARTS = ((0, 6), (6, 2), (8, 1))


def _dot(a, b, dims):
    return jax.lax.dot_general(a, b, dims, preferred_element_type=_F32)


def _ds(i, n):
    return pl.ds(pl.multiple_of(i * n, n), n)


def _start(src, dst, idx, sem, priority):
    pltpu.make_async_copy(src.at[idx], dst.at[idx], sem).start(priority=priority)


def _wait(dst, sem):
    pltpu.make_async_copy(dst, dst, sem).wait()


def _split_heads(src_ref, dst_ref, i):
    inner = src_ref.shape[1]
    w = src_ref[i // inner, i % inner].reshape(_R, H, D)
    dst_ref[_ds(i, _R), :] = w.reshape(_R, H * D)


def _run_pieces(t, pieces):
    first = 0
    for n, every, fn in pieces:
        i = t - first
        pl.when((i >= 0) & (i < n * every) & (i % every == 0))(
            lambda fn=fn, i=i, every=every: fn(i // every))
        first += n * every
    assert first <= _NSTEP


def _kernel(
    ax_hbm, k_hbm, v_hbm, awq_hbm, awo_hbm,
    bx_hbm, ckv_hbm, bwq_hbm, uk_hbm, uv_hbm, bwo_hbm,
    out_ref,
    awq_v, awo_v, ckv_v, bwq_v, uk_v, uv_v, bwo_v,
    ring_v, w2d_v, qa_v, sa_v, oa_v, qb_v, lat_v, pb_v, ob_v, ax_v, bx_v,
    wo_sems,
):
    scale = D ** -0.5

    def b_query(_):
        q = _dot(bx_v[...], w2d_v[...], _NN)
        for h in range(H):
            qb_v[h] = q[:, h * D:(h + 1) * D]

    def b_absorb(h):
        r = _dot(qb_v[h].astype(_BF16), w2d_v[:C, _ds(h, D)], _NT)
        for b in range(B):
            lat_v[pl.ds(b * H + h, 1), :] = r[b:b + 1]

    def ckv(b):
        n = ckv_v.shape[0] // B
        return ckv_v[pl.ds(b * n, n)].reshape(S, C)

    def b_probs(b):
        s = _dot(lat_v[_ds(b, H), :].astype(_BF16), ckv(b), _NT) * scale
        p = jnp.exp(s - jnp.max(s, axis=-1, keepdims=True))
        pb_v[b] = (p / jnp.sum(p, axis=-1, keepdims=True)).astype(_BF16)

    def b_context(b):
        lat_v[_ds(b, H), :] = _dot(pb_v[b], ckv(b), _NN)

    def b_output(h):
        lat = jnp.concatenate(
            [lat_v[pl.ds(b * H + h, 1), :] for b in range(B)], axis=0)
        ctx = _dot(lat.astype(_BF16), w2d_v[:C, _ds(h, D)], _NN)
        n = H // bwo_v.shape[0]
        wo = bwo_v[h // n, pl.ds(pl.multiple_of(h % n * M, 64), M), :]
        ob_v[...] += _dot(ctx.astype(_BF16), wo, _NT)

    def start_wo():
        @pl.loop(0, _R // 8)
        def _(r):
            for q in range(4):
                piece = (_ds(r, 8), pl.ds(q * 1024, 1024))
                _start(awo_hbm, awo_v, (pl.ds(0, 4), *piece), wo_sems.at[0], 1)
                _start(awo_hbm, awo_v, (pl.ds(4, 2), *piece), wo_sems.at[0], 0)

        for j in (1, 2):
            _start(awo_hbm, awo_v, pl.ds(*_WO_PARTS[j]), wo_sems.at[j], 1)

    def stream(sems):
        s_ax, s_bx, s_awq, s_ckv, s_bwq, s_uk, s_uv, s_bwo = (
            sems.at[_NSLOT + i] for i in range(8))

        def start_kv(src, t, slot):
            g, c = t // _NCHUNK, t % _NCHUNK

            @pl.loop(0, _T // 64)
            def _(r):
                for i, n, priority in _FAN:
                    pltpu.make_async_copy(
                        src.at[pl.ds(g * _G + i, n), _ds(c * (_T // 64) + r, 64)],
                        ring_v.at[slot, pl.ds(i, n), _ds(r, 64)],
                        sems.at[slot],
                    ).start(priority=priority)

        pltpu.make_async_copy(ax_hbm, ax_v, s_ax).start()
        pltpu.make_async_copy(bx_hbm, bx_v, s_bx).start()

        @pl.loop(0, 24)
        def _(r):
            for q in range(4):
                p = 4 * r + q
                _start(awq_hbm, awq_v,
                       (_ALL, _ds(r, 8), pl.ds(q * 1024, 1024)), s_awq, 1)
                _start(bwo_hbm, bwo_v, (0, _ds(p, 64)), s_bwo, 0)
                _start(bwq_hbm, bwq_v, (_ALL, p // 32, _ds(p % 32, 64)), s_bwq, 1)
                _start(bwo_hbm, bwo_v, (1, _ds(p, 64)), s_bwo, 0)

        @pl.loop(0, 48)
        def _(p):
            _start(uk_hbm, uk_v, (_ALL, p // 32, _ds(p % 32, 64)), s_uk, 1)
            _start(bwo_hbm, bwo_v, (0, _ds(96 + p, 64)), s_bwo, 0)
            _start(uv_hbm, uv_v, (_ALL, p // 32, _ds(p % 32, 64)), s_uv, 1)
            _start(bwo_hbm, bwo_v, (1, _ds(96 + p, 64)), s_bwo, 0)

        @pl.loop(48, 64)
        def _(p):
            for src, dst, sem in ((uk_hbm, uk_v, s_uk), (uv_hbm, uv_v, s_uv)):
                _start(src, dst, (pl.ds(0, 3), p // 32, _ds(p % 32, 64)), sem, 1)
                _start(src, dst, (3, p // 32, _ds(p % 32, 64)), sem, 0)

        @pl.loop(0, 64)
        def _(p):
            for i, n, priority in _FAN:
                _start(ckv_hbm, ckv_v, (pl.ds(i, n), _ds(p, 16)), s_ckv, priority)

        _wait(ax_v, s_ax)
        _wait(awq_v, s_awq)
        q = _dot(ax_v[...], awq_v[...].reshape(M, H * D), _NN)
        qa_v[...] = q.reshape(B, H, D).reshape(B * H, D)

        @pl.loop(0, _AHEAD)
        def _(t):
            start_kv(k_hbm, t, t)

        _wait(bx_v, s_bx)
        _wait(bwq_v, s_bwq)
        _wait(uk_v, s_uk)
        _wait(uv_v, s_uv)
        _wait(bwo_v, s_bwo)
        _wait(ckv_v, s_ckv)
        ob_v[...] = jnp.zeros(ob_v.shape, ob_v.dtype)

        def each_own_head(lhs, slot, dims):
            out = _dot(lhs, ring_v[slot, 0], dims)
            row = jax.lax.broadcasted_iota(jnp.int32, out.shape, 0)
            for i in range(1, _G):
                out = jnp.where(row == i, _dot(lhs, ring_v[slot, i], dims), out)
            return out

        @pl.loop(0, _NSTEP)
        def _(t):
            nxt = t + _AHEAD
            pl.when(nxt < _NSTEP)(lambda: start_kv(k_hbm, nxt, nxt % _NSLOT))
            pl.when(nxt >= _NSTEP)(
                lambda: start_kv(v_hbm, nxt - _NSTEP, nxt % _NSLOT))
            slot = t % _NSLOT
            _wait(ring_v.at[slot], sems.at[slot])
            q = qa_v[_ds(t // _NCHUNK, _G), :].astype(_BF16)
            sa_v[t] = each_own_head(q, slot, _NT) * scale
            _run_pieces(t, [
                (M // _R, 1, lambda i: _split_heads(bwq_v, w2d_v, i)),
                (1, 1, b_query),
                (C // _R, 1, lambda i: _split_heads(uk_v, w2d_v, i)),
                (H, 1, b_absorb),
            ])

        def v_step(t, carry):
            acc, l = carry
            nxt = t + _AHEAD
            pl.when(nxt < _NSTEP)(
                lambda: start_kv(v_hbm, nxt, (_NSTEP + nxt) % _NSLOT))
            pl.when(nxt == _NSTEP)(start_wo)
            g, c = t // _NCHUNK, t % _NCHUNK
            m = jnp.max(jnp.max(sa_v[pl.ds(g * _NCHUNK, _NCHUNK)], axis=0),
                        axis=-1, keepdims=True)
            p = jnp.exp(sa_v[t] - m)
            l = jnp.where(c == 0, 0.0, l) + jnp.sum(p, axis=-1, keepdims=True)
            slot = (_NSTEP + t) % _NSLOT
            _wait(ring_v.at[slot], sems.at[slot])
            acc = (jnp.where(c == 0, 0.0, acc)
                   + each_own_head(p.astype(_BF16), slot, _NN))

            @pl.when(c == _NCHUNK - 1)
            def _():
                oa_v[_ds(g, _G), :] = acc / l

            _run_pieces(t, [
                (B, 2, b_probs),
                (B, 1, b_context),
                (C // _R, 1, lambda i: _split_heads(uv_v, w2d_v, i)),
                (H, 1, b_output),
            ])
            return acc, l

        jax.lax.fori_loop(0, _NSTEP, v_step,
                          (jnp.zeros((_G, D), _F32), jnp.zeros((_G, 1), _F32)))

    pl.run_scoped(stream, pltpu.SemaphoreType.DMA((_NSLOT + 8,)))

    o = oa_v[...].reshape(B, H, D).reshape(B, H * D).astype(_BF16)
    outs = []
    for j, (i, n) in enumerate(_WO_PARTS):
        _wait(awo_v.at[pl.ds(i, n)], wo_sems.at[j])
        outs.append(_dot(o, awo_v[pl.ds(i, n)].reshape(n * _R, H * D), _NT))
    out_ref[...] = jnp.concatenate(outs + [ob_v[...]], axis=-1).astype(out_ref.dtype)


@jax.jit
def pallas_concat_heads__mha_block_cached__compressed_kv_cla__decode_kernel(
    A_x: jax.Array,
    A_k_cache: jax.Array,
    A_v_cache: jax.Array,
    A_wq: jax.Array,
    A_wo: jax.Array,
    B_x: jax.Array,
    B_c_kv: jax.Array,
    B_w_q: jax.Array,
    B_w_uk: jax.Array,
    B_w_uv: jax.Array,
    B_w_o: jax.Array,
):
    assert A_x.shape == B_x.shape == (B, 1, M)
    assert A_k_cache.shape == A_v_cache.shape == (B, H, S, D)
    assert B_c_kv.shape == (B, S, C)

    ax = A_x.reshape(B, M)
    k = A_k_cache.reshape(B * H, S, D)
    v = A_v_cache.reshape(B * H, S, D)
    awq = A_wq.reshape(3, M // 3, H * D)
    awo = A_wo.T.reshape(M // _R, _R, H * D)
    bx = B_x.reshape(B, M)
    ckv = B_c_kv.reshape(4 * B, S // 4, C)
    bwq = B_w_q.reshape(3, M // _R // 3, _R * H, D)
    uk = B_w_uk.reshape(4, C // _R // 4, _R * H, D)
    uv = B_w_uv.reshape(4, C // _R // 4, _R * H, D)
    bwo = B_w_o.transpose(0, 2, 1).reshape(2, H // 2 * M, D)

    vmem = pltpu.VMEM
    out = pl.pallas_call(
        _kernel,
        out_shape=jax.ShapeDtypeStruct((B, 2 * M), A_x.dtype),
        in_specs=[pl.BlockSpec(memory_space=pltpu.HBM)] * 11,
        out_specs=pl.BlockSpec(memory_space=vmem),
        scratch_shapes=[
            *[vmem(a.shape, _BF16) for a in (awq, awo, ckv, bwq, uk, uv, bwo)],
            vmem((_NSLOT, _G, _T, D), _BF16),
            vmem((M, H * D), _BF16),
            vmem((B * H, D), _F32),
            vmem((_NSTEP, _G, _T), _F32),
            vmem((B * H, D), _F32),
            vmem((H, B, D), _F32),
            vmem((B * H, C), _F32),
            vmem((B, H, S), _BF16),
            vmem((B, M), _F32),
            vmem((B, M), _BF16),
            vmem((B, M), _BF16),
            pltpu.SemaphoreType.DMA((len(_WO_PARTS),)),
        ],
        compiler_params=pltpu.CompilerParams(vmem_limit_bytes=100 * 1024 * 1024),
    )(ax, k, v, awq, awo, bx, ckv, bwq, uk, uv, bwo)
    return out.reshape(B, 1, 2 * M)
```
